```python
import os as _os
_os.environ.setdefault("JAX_PLATFORMS", "cpu")
import jax
import jax.numpy as jnp

def _softmax(x, axis=-1):
    return jax.nn.softmax(x, axis=axis)
def _gelu(x):
    return jax.nn.gelu(x, approximate=True)
def _silu(x):
    return jax.nn.silu(x)
def _sigmoid(x):
    return jax.nn.sigmoid(x)
def _layernorm(x, axis=-1, eps=1e-5):
    m = jnp.mean(x, axis=axis, keepdims=True)
    v = jnp.var(x, axis=axis, keepdims=True)
    return (x - m) / jnp.sqrt(v + eps)
def _scatter_add(tgt, idx, src, axis=0):
    return tgt.at[idx].add(src)
def _segment_sum(src, seg, n):
    return jax.ops.segment_sum(src, seg, n)
class _Rng:
    def __init__(self, key):
        self._k = key
    def _next(self):
        self._k, sub = jax.random.split(self._k)
        return sub
    def normal(self, shape):
        return jax.random.normal(self._next(), shape, dtype=jnp.bfloat16)
    def randint(self, lo, hi, shape):
        return jax.random.randint(self._next(), shape, lo, hi, dtype=jnp.int32)
    def uniform(self, shape, lo=0.0, hi=1.0):
        return jax.random.uniform(self._next(), shape, jnp.bfloat16, lo, hi)
    def permutation(self, n):
        return jax.random.permutation(self._next(), n)


kernel_name = 'standalone__gqa_block_cached__near_ridge'

def setup_inputs():
    _rng = _Rng(jax.random.key(int.from_bytes(__import__("os").urandom(4), "little")))
    _w = (lambda a: (lambda t: t.astype(jnp.bfloat16) if jnp.issubdtype(t.dtype, jnp.floating) else t)(jnp.asarray(a)))
    B, Sq, D = 8, 240, 640
    Hq, Hkv, Sk, Dh = 32, 32, 1024, 192
    assert Hq % Hkv == 0, (Hq, Hkv)
    return {
        "x": _w((lambda *s: _rng.normal(s) * 0.8)(B, Sq, D)),
        "k_cache": _w((lambda *s: _rng.normal(s) * 0.8)(B, Hkv, Sk, Dh)),
        "v_cache": _w((lambda *s: _rng.normal(s) * 0.05)(B, Hkv, Sk, Dh)),
        "wq": _w((lambda *s: _rng.normal(s) * 0.8)(D, Hq * Dh) * (D ** -0.5)),
        "wo": _w((lambda *s: _rng.normal(s) * 0.05)(Hq * Dh, D) * ((Hq * Dh) ** -0.5)),
    }

def reference(x, k_cache, v_cache, wq, wo):
    B, Sq, D = x.shape
    Hq, Dh = 32, 192
    Hkv = k_cache.shape[1]
    rep = Hq // Hkv
    q = (lambda x, *d: x.transpose(*d))((x @ wq).reshape(B, Sq, Hq, Dh), 0, 2, 1, 3)
    k = jnp.repeat(k_cache, rep, axis=1)
    v = jnp.repeat(v_cache, rep, axis=1)
    scores = jnp.einsum("bhqd,bhkd->bhqk", q, k) * (Dh ** -0.5)
    p = _softmax(scores, axis=-1)
    o = jnp.einsum("bhqk,bhkd->bhqd", p, v)
    return (lambda x, *d: x.transpose(*d))(o, 0, 2, 1, 3).reshape(B, Sq, Hq * Dh) @ wo
```

```python
import functools
import math
import os
import jax
import jax.numpy as jnp
from jax import lax
import jax.experimental.pallas as pl
import jax.experimental.pallas.tpu as pltpu

DH = 192
W = 2 * DH
F32 = jnp.float32
BF16 = jnp.bfloat16
U = int(os.environ.get("KU", "4"))
LASTV = int(os.environ.get("KLAST", "1"))
NT = (((1,), (1,)), ((), ()))


def _qproj(x, wq, scale):
    rows = x.shape[0]
    q = jnp.dot(x, wq, preferred_element_type=F32) * scale
    lane = lax.broadcasted_iota(jnp.int32, (rows, 128), 1)
    qm = q[:, 128:256]
    qm1 = jnp.where(lane < 64, qm, 0.0)
    qm2 = jnp.where(lane >= 64, qm, 0.0)
    return jnp.concatenate([q[:, 0:128], qm1, qm2, q[:, 256:384]], axis=1).astype(BF16)


def _softmax(s):
    m = jnp.max(s, axis=1, keepdims=True)
    p = jnp.exp2(s - m)
    nt = s.shape[1] // 128
    parts = [p[:, t * 128:(t + 1) * 128] for t in range(nt)]
    lp = parts[0]
    for t in range(1, nt):
        lp = lp + parts[t]
    l = jnp.sum(lp, axis=1, keepdims=True)
    parts[nt - 1] = jnp.minimum(parts[nt - 1], lp)
    return jnp.concatenate(parts, axis=1).astype(BF16), l


def _kernel(x_hbm, kt_hbm, vt_hbm, wq_hbm, wo_hbm, o_hbm,
            x_buf, kv_buf, wq_buf, wo_buf, acc_ref, q_ref, o_stage, pa_ref, pb_ref,
            x_sem, kv_sem, body_sem, v0_sem, w_sem, o_sem, *, scale, sq, nb, npair):
    ni = nb // U
    lg_u = U.bit_length() - 1
    lg_ni = ni.bit_length() - 1
    lg_nb = nb.bit_length() - 1
    nbody = npair * ni

    def x_copy(g):
        return pltpu.make_async_copy(x_hbm.at[g], x_buf.at[g], x_sem.at[g])

    def kv_one(which, i, sem):
        src = (kt_hbm, vt_hbm)[which]
        if isinstance(i, int):
            pp, g, s, bb = i >> lg_nb, i & (nb - 1), (i >> lg_u) & 1, i & (U - 1)
        else:
            pp = lax.shift_right_logical(i, lg_nb)
            g = jnp.bitwise_and(i, nb - 1)
            s = jnp.bitwise_and(lax.shift_right_logical(i, lg_u), 1)
            bb = jnp.bitwise_and(i, U - 1)
        return pltpu.make_async_copy(src.at[g, pl.ds(pp * W, W)], kv_buf.at[s, which, bb], sem)

    def kv_body(which, it):
        src = (kt_hbm, vt_hbm)[which]
        pp = lax.shift_right_logical(it, lg_ni)
        jj = jnp.bitwise_and(it, ni - 1)
        s = jnp.bitwise_and(it, 1)
        return pltpu.make_async_copy(src.at[pl.ds(jj * U, U), pl.ds(pp * W, W)], kv_buf.at[s, which],
                                     body_sem.at[s])

    def wq_copy(pp):
        s = pp & 1
        return pltpu.make_async_copy(wq_hbm.at[:, pl.ds(pp * W, W)], wq_buf.at[s], w_sem.at[0, s])

    def wo_copy(pp):
        s = pp & 1
        return pltpu.make_async_copy(wo_hbm.at[pl.ds(pp * W, W)], wo_buf.at[s], w_sem.at[1, s])

    def o_copy(g):
        return pltpu.make_async_copy(o_stage.at[g], o_hbm.at[g], o_sem.at[g])

    def attend(slot, bb, g, g_next, wq_slot, wo_slot, z0, z1, mode, hook1=None, hook2=None):
        def qk(h):
            return jnp.dot(q_ref[:, h * 256:(h + 1) * 256],
                           kv_buf[slot, 0, bb, h * 128:h * 128 + 256, :], preferred_element_type=F32)

        def pv(h, pb):
            pr = (pa_ref, pb_ref)[h]
            pr[z0] = pb
            pb = pr[z1]
            od = lax.dot_general(pb, kv_buf[slot, 1, bb, h * 256:h * 256 + 128, :], NT,
                                 preferred_element_type=F32)
            ot = lax.dot_general(kv_buf[slot, 1, bb, 128 + h * 64:192 + h * 64, :], pb, NT,
                                 preferred_element_type=F32)
            return od, ot

        s_a = qk(0)
        s_b = qk(1)
        if hook1 is not None:
            hook1()
        p_a, l_a = _softmax(s_a)
        o_a = pv(0, p_a)
        p_b, l_b = _softmax(s_b)
        o_b = pv(1, p_b)
        if hook2 is not None:
            hook2()
        q_ref[...] = _qproj(x_buf[g_next], wq_buf[wq_slot], scale)
        lane = lax.broadcasted_iota(jnp.int32, (sq, 128), 1)
        ia = 1.0 / l_a
        ib = 1.0 / l_b
        om = jnp.concatenate([o_a[1], o_b[1]], axis=0).T
        o = jnp.concatenate(
            [o_a[0] * ia, om * jnp.where(lane < 64, ia, ib), o_b[0] * ib], axis=1).astype(BF16)
        contrib = jnp.dot(o, wo_buf[wo_slot], preferred_element_type=F32)
        if mode == "first":
            acc_ref[g] = contrib
        elif mode == "last":
            o_stage[g] = (acc_ref[g] + contrib).astype(o_stage.dtype)
            o_copy(g).start()
        else:
            acc_ref[g] += contrib

    n_ramp_loads = nb + U

    def kv_sem_for(i):
        if isinstance(i, int):
            return kv_sem.at[i] if i < nb else body_sem.at[(i >> lg_u) & 1]
        raise AssertionError

    zero = pl.program_id(0)
    x_copy(0).start()
    wq_copy(0).start()
    kv_one(0, 0, kv_sem.at[0]).start()
    x_copy(0).wait()
    wq_copy(0).wait()
    kv_one(1, 0, v0_sem.at[0]).start()
    q_ref[...] = _qproj(x_buf[0], wq_buf[0], scale)
    kv_one(0, 0, kv_sem.at[0]).wait()
    x_copy(1).start()
    wo_copy(0).start()

    def hook1():
        kv_one(1, 0, v0_sem.at[0]).wait()
        kv_one(0, 1, kv_sem_for(1)).start()
        kv_one(1, 1, kv_sem_for(1)).start()
        x_copy(2).start()

    H2 = int(os.environ.get("KH2", "0"))
    PER = int(os.environ.get("KPER", "3"))
    halves = [(w, i) for i in range(2, n_ramp_loads) for w in (0, 1)]

    def hook2():
        x_copy(1).wait()
        wo_copy(0).wait()
        for w, i in halves[:H2]:
            kv_one(w, i, kv_sem_for(i)).start()

    attend(0, 0, 0, 1, 0, 0, zero, zero * 2, "first", hook1, hook2)

    sched = {}
    pos = H2
    for g in range(1, nb):
        budget = PER - 1 if g == nb - 2 else PER
        if g == nb - 1:
            budget = len(halves)
        items = []
        while pos < len(halves) and len(items) < budget and halves[pos][1] <= g + 2 * U - 1:
            items.append(halves[pos])
            pos += 1
        sched[g] = items
        assert all(i > g + 1 for _, i in halves[pos:]) or g + 1 >= nb
    assert pos == len(halves), sched

    def ramp_body(g, carry):
        sem = kv_sem.at[g]
        kv_one(0, g, sem).wait()
        kv_one(1, g, sem).wait()

        @pl.when(g + 1 < nb)
        def _():
            x_copy(g + 1).wait()

        @pl.when(g + 1 == nb)
        def _():
            wq_copy(1).wait()
            wo_copy(1).wait()

        for gg, loads in sched.items():
            @pl.when(g == gg)
            def _():
                for w, i in loads:
                    kv_one(w, i, kv_sem_for(i)).start()
                if gg + 2 < nb:
                    x_copy(gg + 2).start()
                if gg == nb - 2:
                    wq_copy(1).start()
                    wo_copy(1).start()

        slot = jnp.bitwise_and(lax.shift_right_logical(g, lg_u), 1)
        bb = jnp.bitwise_and(g, U - 1)
        g_next = jnp.bitwise_and(g + 1, nb - 1)
        wq_slot = lax.shift_right_logical(g + 1, lg_nb)
        attend(slot, bb, g, g_next, wq_slot, 0, lax.shift_right_logical(g, 10),
               lax.shift_right_logical(g, 11), "first")
        return carry

    lax.fori_loop(1, nb, ramp_body, 0)
    if ni + 1 < nbody:
        kv_body(0, ni + 1).start()
        kv_body(1, ni + 1).start()
    if npair > 2:
        wq_copy(2).start()
        wo_copy(2).start()

    def fast_body(mode, it, carry):
        p = lax.shift_right_logical(it, lg_ni)
        j = jnp.bitwise_and(it, ni - 1)
        slot = jnp.bitwise_and(it, 1)
        last_j = j == ni - 1
        pltpu.make_async_copy(kv_buf.at[slot], kv_buf.at[slot], body_sem.at[slot]).wait()
        if mode != "last":
            @pl.when(jnp.logical_and(last_j, p + 1 < npair))
            def _():
                wq_copy(p + 1).wait()
                wo_copy(p + 1).wait()

        z0 = lax.shift_right_logical(it, 10)
        z1 = lax.shift_right_logical(it, 11)
        ps = jnp.bitwise_and(p, 1)
        for bb in range(U):
            g = j * U + bb
            if bb + 1 < U:
                g_next, wq_slot = g + 1, ps
            else:
                g_next = jnp.bitwise_and(g + 1, nb - 1)
                pq = jnp.minimum(lax.shift_right_logical(it + 1, lg_ni), npair - 1)
                wq_slot = jnp.bitwise_and(pq, 1)
            attend(slot, bb, g, g_next, wq_slot, ps, z0, z1, mode)

        @pl.when(it + 2 < nbody)
        def _():
            kv_body(0, it + 2).start()
            kv_body(1, it + 2).start()

        if mode != "last":
            @pl.when(jnp.logical_and(last_j, p + 2 < npair))
            def _():
                wq_copy(p + 2).start()
                wo_copy(p + 2).start()
        return carry

    if LASTV:
        lax.fori_loop(ni, nbody - ni, functools.partial(fast_body, "mid"), 0)
        lax.fori_loop(nbody - ni, nbody, functools.partial(fast_body, "last"), 0)
    else:
        lax.fori_loop(ni, nbody, functools.partial(fast_body, "mid"), 0)
        for g in range(nb):
            o_stage[g] = acc_ref[g].astype(o_stage.dtype)
            o_copy(g).start()
    for g in range(nb):
        o_copy(g).wait()


@jax.jit
def pallas_standalone__gqa_block_cached__near_ridge_kernel(x, k_cache, v_cache, wq, wo):
    B, Sq, D = x.shape
    _, Hkv, Sk, Dh = k_cache.shape
    kt = jnp.swapaxes(k_cache, 2, 3).reshape(B, Hkv * Dh, Sk)
    vt = jnp.swapaxes(v_cache, 2, 3).reshape(B, Hkv * Dh, Sk)
    scale = (Dh ** -0.5) * math.log2(math.e)
    npair = int(os.environ.get("KNP", Hkv // 2))
    any_spec = pl.BlockSpec(memory_space=pl.ANY)
    return pl.pallas_call(
        functools.partial(_kernel, scale=scale, sq=Sq, nb=B, npair=npair),
        grid=(1,),
        in_specs=[any_spec] * 5,
        out_specs=any_spec,
        out_shape=jax.ShapeDtypeStruct((B, Sq, D), x.dtype),
        scratch_shapes=[
            pltpu.VMEM((B, Sq, D), BF16),
            pltpu.VMEM((2, 2, U, W, Sk), BF16),
            pltpu.VMEM((2, D, W), BF16),
            pltpu.VMEM((2, W, D), BF16),
            pltpu.VMEM((B, Sq, D), F32),
            pltpu.VMEM((Sq, 512), BF16),
            pltpu.VMEM((B, Sq, D), BF16),
            pltpu.VMEM((1, Sq, Sk), BF16),
            pltpu.VMEM((1, Sq, Sk), BF16),
            pltpu.SemaphoreType.DMA((B,)),
            pltpu.SemaphoreType.DMA((B,)),
            pltpu.SemaphoreType.DMA((2,)),
            pltpu.SemaphoreType.DMA((1,)),
            pltpu.SemaphoreType.DMA((2, 2)),
            pltpu.SemaphoreType.DMA((B,)),
        ],
        compiler_params=pltpu.CompilerParams(
            dimension_semantics=("arbitrary",),
            vmem_limit_bytes=100 * 1024 * 1024,
            disable_bounds_checks=True,
        ),
    )(x, kt, vt, wq, wo)
```

```python
import functools
import math
import jax
import jax.numpy as jnp
from jax import lax
import jax.experimental.pallas as pl
import jax.experimental.pallas.tpu as pltpu

DH = 192
W = 2 * DH
GW = 2 * W
F32 = jnp.float32
BF16 = jnp.bfloat16
NT = (((1,), (1,)), ((), ()))
Q_ORDER = "b537a142c6d"
O_ORDER = "ab3571426"
O_ORDER_FINAL = "a3561247b"
K_ORDER = ('3', '1246', '57')


def _dot(a, b):
    return jnp.dot(a, b, preferred_element_type=F32)


def _add(a, b):
    return (a.astype(F32) + b.astype(F32)).astype(BF16)


def _sub(a, b):
    return (a.astype(F32) - b.astype(F32)).astype(BF16)


def _softmax(s):
    m = jnp.max(s, axis=1, keepdims=True)
    p = jnp.exp2(s - m)
    nt = s.shape[1] // 128
    parts = [p[:, t * 128:(t + 1) * 128] for t in range(nt)]
    lp = parts[0]
    for t in range(1, nt):
        lp = lp + parts[t]
    l = jnp.sum(lp, axis=1, keepdims=True)
    parts[nt - 1] = jnp.minimum(parts[nt - 1], lp)
    return jnp.concatenate(parts, axis=1).astype(BF16), l


def _rcp(l):
    r = pl.reciprocal(l, approx=True)
    return r * (2.0 - l * r)


def _kernel(x_hbm, kt_hbm, vt_hbm, wq_hbm, wo_hbm, o_hbm,
            x_buf, kv_buf, wq_buf, wo_buf, acc_ref, q_ref, o_stage, pa_ref, pb_ref, o_ref, zs,
            x_sem, kv_sem, body_sem, f_sem, w_sem, o_sem, *, scale, sq, nb, ngroup):
    ni = nb // 2
    lg_ni = ni.bit_length() - 1
    nbody = ngroup * ni
    d_model = x_buf.shape[2]
    kh = (d_model // 256) * 128
    lane = lax.broadcasted_iota(jnp.int32, (sq, 128), 1)

    def x_copy(g):
        return pltpu.make_async_copy(x_hbm.at[g], x_buf.at[g], x_sem.at[g])

    def kv_step(which, i, sem):
        src = (kt_hbm, vt_hbm)[which]
        it, bi, pi = i // 4, (i >> 1) & 1, i & 1
        gg, jj = it // ni, it % ni
        return pltpu.make_async_copy(src.at[2 * jj + bi, pl.ds(gg * GW + pi * W, W)],
                                     kv_buf.at[it & 1, which, bi, pl.ds(pi * W, W)], sem)

    def kv_body(which, it):
        src = (kt_hbm, vt_hbm)[which]
        gg = lax.shift_right_logical(it, lg_ni)
        jj = jnp.bitwise_and(it, ni - 1)
        s = jnp.bitwise_and(it, 1)
        return pltpu.make_async_copy(src.at[pl.ds(jj * 2, 2), pl.ds(gg * GW, GW)], kv_buf.at[s, which],
                                     body_sem.at[s])

    def wq_copy(gg, pi):
        s = gg & 1
        return pltpu.make_async_copy(wq_hbm.at[:, pl.ds(gg * GW + pi * W, W)], wq_buf.at[s, pi],
                                     w_sem.at[pi, s])

    def wo_copy(gg):
        s = gg & 1
        return pltpu.make_async_copy(wo_hbm.at[pl.ds(gg * GW, GW)], wo_buf.at[s], w_sem.at[2, s])

    def o_copy(g):
        return pltpu.make_async_copy(o_stage.at[g], o_hbm.at[g], o_sem.at[g])

    def o_part(g, c0, c1):
        return pltpu.make_async_copy(o_stage.at[g, :, pl.ds(c0, c1 - c0)], o_hbm.at[g, :, pl.ds(c0, c1 - c0)],
                                     o_sem.at[g])

    r2 = sq - 128

    def store_q(st, q):
        q = q * scale
        qm = q[:, 128:256]
        tiles = [q[:, 0:128], jnp.where(lane < 64, qm, 0.0), jnp.where(lane >= 64, qm, 0.0), q[:, 256:384]]
        for h in range(2):
            t0, t1 = tiles[2 * h], tiles[2 * h + 1]
            a11, a12, a21, a22 = t0[0:128], t1[0:128], t0[128:], t1[128:]
            full = jnp.concatenate([
                jnp.concatenate([a11[0:r2] + a22, a11[r2:]], axis=0),
                a11,
                a11 + a12,
                jnp.concatenate([a12[0:r2] - a22, a12[r2:]], axis=0),
            ], axis=1)
            part = jnp.concatenate([a21 + a22, a22, a21 - a11[0:r2]], axis=1)
            q_ref[st, 0:128, h * 512:(h + 1) * 512] = full.astype(BF16)
            q_ref[st, 128:, h * 512:h * 512 + 384] = part.astype(BF16)

    def combine(terms):
        first = next(i for i, e in enumerate(terms) if e[1] > 0)
        tot = terms[first][0]
        for i, (v, sg) in enumerate(terms):
            if i != first:
                tot = tot + v if sg > 0 else tot - v
        return tot

    def qproj_group(g0, ws):
        zz = [0, zs[0], zs[1], zs[2]]

        def xa(i, k, v):
            return x_buf[g0 + i + zz[v], :, k * kh:min((k + 1) * kh, d_model)]

        def wb(k, j, v):
            return wq_buf[ws + zz[v], j, k * kh:min((k + 1) * kh, d_model), :]

        prods = {
            "1": lambda: _dot(_add(xa(0, 0, 0), xa(1, 1, 0)), _add(wb(0, 0, 0), wb(1, 1, 0))),
            "2": lambda: _dot(_add(xa(1, 0, 0), xa(1, 1, 1)), wb(0, 0, 1)),
            "3": lambda: _dot(xa(0, 0, 1), _sub(wb(0, 1, 0), wb(1, 1, 1))),
            "4": lambda: _dot(xa(1, 1, 2), _sub(wb(1, 0, 0), wb(0, 0, 2))),
            "5": lambda: _dot(_add(xa(0, 0, 2), xa(0, 1, 0)), wb(1, 1, 2)),
            "6": lambda: _dot(_sub(xa(1, 0, 1), xa(0, 0, 3)), _add(wb(0, 0, 3), wb(0, 1, 1))),
            "7": lambda: _dot(_sub(xa(0, 1, 1), xa(1, 1, 3)), _add(wb(1, 0, 1), wb(1, 1, 3))),
            "a": lambda: _dot(xa(0, 2, 0), wb(2, 0, 0)),
            "b": lambda: _dot(xa(0, 2, 1), wb(2, 1, 0)),
            "c": lambda: _dot(xa(1, 2, 0), wb(2, 0, 1)),
            "d": lambda: _dot(xa(1, 2, 1), wb(2, 1, 1)),
        }
        uses = {"1": ((0, 1), (3, 1)), "2": ((2, 1), (3, -1)), "3": ((1, 1), (3, 1)), "4": ((0, 1), (2, 1)),
                "5": ((0, -1), (1, 1)), "6": ((3, 1),), "7": ((0, 1),),
                "a": ((0, 1),), "b": ((1, 1),), "c": ((2, 1),), "d": ((3, 1),)}
        need = [5, 3, 3, 5]
        pend = [[], [], [], []]
        for t in Q_ORDER:
            m = prods[t]()
            for st, sg in uses[t]:
                pend[st].append((m, sg))
                if len(pend[st]) == need[st]:
                    tot = combine(pend[st])
                    store_q(st, tot)

    def oproj_group(g0, ws, last, static_out=False):
        zz = [zs[0], zs[1], zs[2], zs[3], zs[4]]
        zw = [0, zs[0], zs[1], zs[2]]

        def emit(g, c0, c1, val):
            tot = acc_ref[g, :, c0:c1] + val
            if last:
                o_stage[g, :, c0:c1] = tot.astype(o_stage.dtype)
                if static_out:
                    o_part(g, c0, c1).start()
            else:
                acc_ref[g, :, c0:c1] = tot

        def oa(i, k, v):
            return o_ref[2 * i + k + (0 if static_out else zz[v])]

        def wb(k, j, v):
            return wo_buf[ws + zw[v], k * W:(k + 1) * W, j * kh:min((j + 1) * kh, d_model)]

        bf = lambda v: v.astype(BF16)
        prods = {
            "1": lambda: _dot(bf(oa(0, 0, 0) + oa(1, 1, 0)), _add(wb(0, 0, 0), wb(1, 1, 0))),
            "2": lambda: _dot(bf(oa(1, 0, 0) + oa(1, 1, 1)), wb(0, 0, 1)),
            "3": lambda: _dot(bf(oa(0, 0, 1)), _sub(wb(0, 1, 0), wb(1, 1, 1))),
            "4": lambda: _dot(bf(oa(1, 1, 2)), _sub(wb(1, 0, 0), wb(0, 0, 2))),
            "5": lambda: _dot(bf(oa(0, 0, 2) + oa(0, 1, 0)), wb(1, 1, 2)),
            "6": lambda: _dot(bf(oa(1, 0, 1) - oa(0, 0, 3)), _add(wb(0, 0, 3), wb(0, 1, 1))),
            "7": lambda: _dot(bf(oa(0, 1, 1) - oa(1, 1, 3)), _add(wb(1, 0, 1), wb(1, 1, 3))),
            "a": lambda: _dot(bf(jnp.concatenate([oa(0, 0, 4), oa(0, 1, 2)], axis=1)), wo_buf[ws, :, 2 * kh:]),
            "b": lambda: _dot(bf(jnp.concatenate([oa(1, 0, 2), oa(1, 1, 4)], axis=1)), wo_buf[ws + zw[1], :, 2 * kh:]),
        }
        uses = {"1": ((0, 1), (3, 1)), "2": ((2, 1), (3, -1)), "3": ((1, 1), (3, 1)), "4": ((0, 1), (2, 1)),
                "5": ((0, -1), (1, 1)), "6": ((3, 1),), "7": ((0, 1),), "a": ((4, 1),), "b": ((5, 1),)}
        need = [4, 2, 2, 4, 1, 1]
        dest = [(0, 0), (0, 1), (1, 0), (1, 1), (0, 2), (1, 2)]
        pend = [[] for _ in need]
        for t in (O_ORDER_FINAL if static_out else O_ORDER):
            m = prods[t]()
            for st, sg in uses[t]:
                pend[st].append((m, sg))
                if len(pend[st]) == need[st]:
                    tot = combine(pend[st])
                    bi, jj = dest[st]
                    emit(g0 + bi, jj * kh, min((jj + 1) * kh, d_model), tot)
        if last and not static_out:
            o_copy(g0).start()
            o_copy(g0 + 1).start()

    def attend(slot, st, z0, z1):
        bi, r = st >> 1, (st & 1) * W
        if not isinstance(st, int):
            r = pl.multiple_of(r, 128)

        def rows(a, n):
            return pl.ds(r + a, n)

        def qk(h):
            zz = [0, zs[2], zs[3], zs[4]] if h == 0 else [zs[5], zs[6], zs[7], zs[8]]
            cw = 128
            half = kv_buf.shape[4] // 2

            def kb(d, j, c, v):
                return kv_buf[slot + zz[v], 0, bi, rows((h + d) * 128, 128), j * half + c:j * half + c + cw]

            def qa(m):
                if m % 2:
                    return q_ref[st, 0:128, h * 512 + (m // 2) * 128:h * 512 + (m // 2 + 1) * 128]
                return q_ref[st, 128:, h * 512 + (m // 2 - 1) * 128:h * 512 + (m // 2) * 128]

            def prod(t, c):
                return {
                    1: lambda: _dot(qa(1), _add(kb(0, 0, c, 0), kb(1, 1, c, 0))),
                    2: lambda: _dot(qa(2), kb(0, 0, c, 1)),
                    3: lambda: _dot(qa(3), _sub(kb(0, 1, c, 0), kb(1, 1, c, 1))),
                    4: lambda: _dot(qa(4), _sub(kb(1, 0, c, 0), kb(0, 0, c, 2))),
                    5: lambda: _dot(qa(5), kb(1, 1, c, 2)),
                    6: lambda: _dot(qa(6), _add(kb(0, 0, c, 3), kb(0, 1, c, 1))),
                    7: lambda: _dot(qa(7), _add(kb(1, 0, c, 1), kb(1, 1, c, 3))),
                }[t]()

            cs = list(range(0, half, cw))
            m = {}
            for phase in K_ORDER:
                for c in cs:
                    for t in phase:
                        m[int(t), c] = prod(int(t), c)
            c11, c12, c21, c22 = [], [], [], []
            for c in cs:
                w_ = jnp.concatenate([m[1, c][0:r2] + m[4, c], m[1, c][r2:]], axis=0)
                c11.append(w_ + (m[7, c] - m[5, c]))
                c22.append(m[1, c][0:r2] - m[2, c] + m[6, c] + m[3, c][0:r2])
                c12.append(m[3, c] + m[5, c])
                c21.append(m[2, c] + m[4, c])
            return jnp.concatenate([jnp.concatenate(c11 + c12, axis=1), jnp.concatenate(c21 + c22, axis=1)], axis=0)

        def pv(h, s):
            pb, l = _softmax(s)
            pr = (pa_ref, pb_ref)[h]
            pr[z0] = pb
            ot = lax.dot_general(kv_buf[slot, 1, bi, rows(128 + h * 64, 64), :], pr[zs[2]], NT,
                                 preferred_element_type=F32)
            od = lax.dot_general(pr[z1], kv_buf[slot, 1, bi, rows(h * 256, 128), :], NT,
                                 preferred_element_type=F32)
            return od, ot, _rcp(l)

        def fin(ra, rb):
            od_a, ot_a, ia = ra
            od_b, ot_b, ib = rb
            om = jnp.concatenate([ot_a, ot_b], axis=0).T
            o_ref[st] = jnp.concatenate([od_a * ia, om * jnp.where(lane < 64, ia, ib), od_b * ib], axis=1)

        return qk, pv, fin

    def attend_seq(slot, sts, z0, z1):
        parts = [attend(slot, st, z0, z1) for st in sts]
        n = 2 * len(sts)
        s = {}
        r = {}
        seq = ["K0"]
        for u in range(n):
            if u + 1 < n:
                seq.append("K%d" % (u + 1))
            seq.append("P%d" % u)
        for tok in seq:
            u = int(tok[1:])
            qk, pv, fin = parts[u // 2]
            if tok[0] == "K":
                s[u] = qk(u % 2)
            else:
                r[u] = pv(u % 2, s[u])
                if u % 2 == 1:
                    fin(r[u - 1], r[u])

    def kv(i):
        return [functools.partial(kv_step, 0, i, kv_sem.at[i]), functools.partial(kv_step, 1, i, kv_sem.at[i])]

    def xs(*gs):
        return [functools.partial(x_copy, g) for g in gs]

    def start(mks):
        for mk in mks:
            mk().start()

    def wait(mks):
        for mk in mks:
            mk().wait()

    def fence():
        pl.semaphore_signal(f_sem, 1)
        pl.semaphore_wait(f_sem, 1)

    wq00, wq01 = [functools.partial(wq_copy, 0, 0)], [functools.partial(wq_copy, 0, 1)]
    wo0 = [functools.partial(wo_copy, 0)]
    w1 = [functools.partial(wq_copy, 1, 0), functools.partial(wq_copy, 1, 1), functools.partial(wo_copy, 1)]
    for i in range(9):
        zs[i] = 0

    def at(i, table, fn):
        for key, mks in table.items():
            if mks:
                pl.when(i == key)(functools.partial(fn, mks))

    for group in (xs(0) + wq00, xs(1), wq01, kv(0) + kv(1) + kv(2) + kv(3), xs(2, 3), wo0,
                  kv(4) + kv(5) + kv(6) + kv(7), xs(4, 5)):
        start(group)
        fence()

    def zero_body(g, carry):
        acc_ref[g] = jnp.zeros(acc_ref.shape[1:], F32)
        return carry

    lax.fori_loop(0, nb, zero_body, 0)

    def q0_body(i, carry):
        at(i, {0: xs(0) + wq00, 1: xs(1), 2: wq01}, wait)
        g = jnp.bitwise_and(i, 1)
        pi = lax.shift_right_logical(i, 1)
        store_q(2 * g + pi, _dot(x_buf[g], wq_buf[0, pi]))
        return carry

    lax.fori_loop(0, 4, q0_body, 0)

    def ramp_body(i, carry):
        slot = lax.shift_right_logical(i, 2)
        st = jnp.bitwise_and(i, 3)
        for which in range(2):
            dst = kv_buf.at[slot, which, lax.shift_right_logical(st, 1),
                            pl.ds(pl.multiple_of(jnp.bitwise_and(st, 1) * W, 128), W)]
            pltpu.make_async_copy(dst, dst, kv_sem.at[i]).wait()
        attend_seq(slot, [st], zs[0], zs[1])

        @pl.when(st == 3)
        def _():
            kv_body(0, slot + 2).start()
            kv_body(1, slot + 2).start()
            at(i, {3: xs(2, 3) + wo0, 7: xs(4, 5)}, wait)
            at(i, {3: xs(6, 7), 7: w1}, start)
            fence()
            qproj_group(2 * slot + 2, 0)
            oproj_group(2 * slot, 0, False)
        return carry

    lax.fori_loop(0, 8, ramp_body, 0)
    wait(xs(6, 7))

    def fast_body(mode, it, carry):
        gg = lax.shift_right_logical(it, lg_ni)
        j = jnp.bitwise_and(it, ni - 1)
        slot = jnp.bitwise_and(it, 1)
        last_j = j == ni - 1
        pltpu.make_async_copy(kv_buf.at[slot], kv_buf.at[slot], body_sem.at[slot]).wait()
        if mode == "mid":
            @pl.when(last_j)
            def _():
                wq_copy(gg + 1, 0).wait()
                wq_copy(gg + 1, 1).wait()
                wo_copy(gg + 1).wait()

        z0, z1 = zs[0], zs[1]
        attend_seq(slot, [0, 1, 2, 3], z0, z1)
        if mode != "final":
            gq = jnp.minimum(lax.shift_right_logical(it + 1, lg_ni), ngroup - 1)
            qproj_group(2 * jnp.bitwise_and(it + 1, ni - 1), jnp.bitwise_and(gq, 1))
        if mode == "final":
            oproj_group(nb - 2, (ngroup - 1) & 1, True, True)
        else:
            oproj_group(2 * j, jnp.bitwise_and(gg, 1), mode != "mid")

        if mode != "final":
            @pl.when(it + 2 < nbody)
            def _():
                kv_body(0, it + 2).start()
                kv_body(1, it + 2).start()

        if mode == "mid":
            @pl.when(jnp.logical_and(last_j, gg + 2 < ngroup))
            def _():
                wq_copy(gg + 2, 0).start()
                wq_copy(gg + 2, 1).start()
                wo_copy(gg + 2).start()
        return carry

    lax.fori_loop(2, nbody - ni, functools.partial(fast_body, "mid"), 0)
    lax.fori_loop(nbody - ni, nbody - 1, functools.partial(fast_body, "last"), 0)
    fast_body("final", jnp.int32(nbody - 1), 0)
    for g in range(nb):
        o_copy(g).wait()


@jax.jit
def pallas_standalone__gqa_block_cached__near_ridge_kernel(x, k_cache, v_cache, wq, wo):
    B, Sq, D = x.shape
    _, Hkv, Sk, Dh = k_cache.shape
    kt = jnp.swapaxes(k_cache, 2, 3).reshape(B, Hkv * Dh, Sk)
    vt = jnp.swapaxes(v_cache, 2, 3).reshape(B, Hkv * Dh, Sk)
    scale = (Dh ** -0.5) * math.log2(math.e)
    ngroup = Hkv // 4
    any_spec = pl.BlockSpec(memory_space=pl.ANY)
    return pl.pallas_call(
        functools.partial(_kernel, scale=scale, sq=Sq, nb=B, ngroup=ngroup),
        grid=(1,),
        in_specs=[any_spec] * 5,
        out_specs=any_spec,
        out_shape=jax.ShapeDtypeStruct((B, Sq, D), x.dtype),
        scratch_shapes=[
            pltpu.VMEM((B, Sq, D), BF16),
            pltpu.VMEM((2, 2, 2, GW, Sk), BF16),
            pltpu.VMEM((2, 2, D, W), BF16),
            pltpu.VMEM((2, GW, D), BF16),
            pltpu.VMEM((B, Sq, D), F32),
            pltpu.VMEM((4, Sq, 1024), BF16),
            pltpu.VMEM((B, Sq, D), BF16),
            pltpu.VMEM((1, Sq, Sk), BF16),
            pltpu.VMEM((1, Sq, Sk), BF16),
            pltpu.VMEM((4, Sq, W), F32),
            pltpu.SMEM((9,), jnp.int32),
            pltpu.SemaphoreType.DMA((B,)),
            pltpu.SemaphoreType.DMA((8,)),
            pltpu.SemaphoreType.DMA((2,)),
            pltpu.SemaphoreType.REGULAR,
            pltpu.SemaphoreType.DMA((3, 2)),
            pltpu.SemaphoreType.DMA((B,)),
        ],
        compiler_params=pltpu.CompilerParams(
            dimension_semantics=("arbitrary",),
            vmem_limit_bytes=100 * 1024 * 1024,
            disable_bounds_checks=True,
        ),
    )(x, kt, vt, wq, wo)
```

```python
import functools
import math
import jax
import jax.numpy as jnp
from jax import lax
import jax.experimental.pallas as pl
import jax.experimental.pallas.tpu as pltpu

DH = 192
W = 2 * DH
GW = 2 * W
F32 = jnp.float32
BF16 = jnp.bfloat16
NT = (((1,), (1,)), ((), ()))
Q_ORDER = "53b7a142c6d"
O_ORDER = "3571426"
O_ORDER_TAIL = "ab"
O_ORDER_FINAL = "a3561247b"
K_ORDER = ("3", "1246", "57")
K_ORDER_FIRST = ("2", "3146", "57")


def _dot(a, b):
    return jnp.dot(a, b, preferred_element_type=F32)


def _add(a, b):
    return (a.astype(F32) + b.astype(F32)).astype(BF16)


def _sub(a, b):
    return (a.astype(F32) - b.astype(F32)).astype(BF16)


def _softmax(s):
    m = jnp.max(s, axis=1, keepdims=True)
    p = jnp.exp2(s - m)
    nt = s.shape[1] // 128
    parts = [p[:, t * 128:(t + 1) * 128] for t in range(nt)]
    lp = parts[0]
    for t in range(1, nt):
        lp = lp + parts[t]
    l = jnp.sum(lp, axis=1, keepdims=True)
    parts[nt - 1] = jnp.minimum(parts[nt - 1], lp)
    return jnp.concatenate(parts, axis=1).astype(BF16), l


def _rcp(l):
    r = pl.reciprocal(l, approx=True)
    return r * (2.0 - l * r)


def _kernel(x_hbm, kt_hbm, vt_hbm, wq_hbm, wo_hbm, o_hbm,
            x_buf, kv_buf, wq_buf, wo_buf, acc_ref, q_ref, o_stage, pa_ref, pb_ref, o_ref, zs,
            x_sem, kv_sem, body_sem, f_sem, w_sem, o_sem, *, scale, sq, nb, ngroup):
    ni = nb // 2
    lg_ni = ni.bit_length() - 1
    nbody = ngroup * ni
    d_model = x_buf.shape[2]
    kh = (d_model // 256) * 128
    lane = lax.broadcasted_iota(jnp.int32, (sq, 128), 1)

    def x_copy(g):
        return pltpu.make_async_copy(x_hbm.at[g], x_buf.at[g], x_sem.at[g])

    def kv_step(which, i, sem):
        src = (kt_hbm, vt_hbm)[which]
        it, bi, pi = i // 4, (i >> 1) & 1, i & 1
        gg, jj = it // ni, it % ni
        return pltpu.make_async_copy(src.at[2 * jj + bi, pl.ds(gg * GW + pi * W, W)],
                                     kv_buf.at[it & 1, which, bi, pl.ds(pi * W, W)], sem)

    def kv_body(which, it):
        src = (kt_hbm, vt_hbm)[which]
        gg = lax.shift_right_logical(it, lg_ni)
        jj = jnp.bitwise_and(it, ni - 1)
        s = jnp.bitwise_and(it, 1)
        return pltpu.make_async_copy(src.at[pl.ds(jj * 2, 2), pl.ds(gg * GW, GW)], kv_buf.at[s, which],
                                     body_sem.at[s])

    def wq_copy(gg, pi):
        s = gg & 1
        return pltpu.make_async_copy(wq_hbm.at[:, pl.ds(gg * GW + pi * W, W)], wq_buf.at[s, pi],
                                     w_sem.at[pi, s])

    def wo_copy(gg):
        s = gg & 1
        return pltpu.make_async_copy(wo_hbm.at[pl.ds(gg * GW, GW)], wo_buf.at[s], w_sem.at[2, s])

    def o_copy(g):
        return pltpu.make_async_copy(o_stage.at[g], o_hbm.at[g], o_sem.at[g])

    def o_part(g, c0, c1):
        return pltpu.make_async_copy(o_stage.at[g, :, pl.ds(c0, c1 - c0)], o_hbm.at[g, :, pl.ds(c0, c1 - c0)],
                                     o_sem.at[g])

    r2 = sq - 128

    def store_q(st, q):
        q = q * scale
        qm = q[:, 128:256]
        tiles = [q[:, 0:128], jnp.where(lane < 64, qm, 0.0), jnp.where(lane >= 64, qm, 0.0), q[:, 256:384]]
        for h in range(2):
            t0, t1 = tiles[2 * h], tiles[2 * h + 1]
            a11, a12, a21, a22 = t0[0:128], t1[0:128], t0[128:], t1[128:]
            full = jnp.concatenate([
                jnp.concatenate([a11[0:r2] + a22, a11[r2:]], axis=0),
                a11,
                a11 + a12,
                jnp.concatenate([a12[0:r2] - a22, a12[r2:]], axis=0),
            ], axis=1)
            part = jnp.concatenate([a21 + a22, a22, a21 - a11[0:r2]], axis=1)
            q_ref[st, 0:128, h * 512:(h + 1) * 512] = full.astype(BF16)
            q_ref[st, 128:, h * 512:h * 512 + 384] = part.astype(BF16)

    def combine(terms):
        first = next(i for i, e in enumerate(terms) if e[1] > 0)
        tot = terms[first][0]
        for i, (v, sg) in enumerate(terms):
            if i != first:
                tot = tot + v if sg > 0 else tot - v
        return tot

    def qproj_group(g0, ws):
        zz = [0, zs[0], zs[1], zs[2]]

        def xa(i, k, v):
            return x_buf[g0 + i + zz[v], :, k * kh:min((k + 1) * kh, d_model)]

        def wb(k, j, v):
            return wq_buf[ws + zz[v], j, k * kh:min((k + 1) * kh, d_model), :]

        prods = {
            "1": lambda: _dot(_add(xa(0, 0, 0), xa(1, 1, 0)), _add(wb(0, 0, 0), wb(1, 1, 0))),
            "2": lambda: _dot(_add(xa(1, 0, 0), xa(1, 1, 1)), wb(0, 0, 1)),
            "3": lambda: _dot(xa(0, 0, 1), _sub(wb(0, 1, 0), wb(1, 1, 1))),
            "4": lambda: _dot(xa(1, 1, 2), _sub(wb(1, 0, 0), wb(0, 0, 2))),
            "5": lambda: _dot(_add(xa(0, 0, 2), xa(0, 1, 0)), wb(1, 1, 2)),
            "6": lambda: _dot(_sub(xa(1, 0, 1), xa(0, 0, 3)), _add(wb(0, 0, 3), wb(0, 1, 1))),
            "7": lambda: _dot(_sub(xa(0, 1, 1), xa(1, 1, 3)), _add(wb(1, 0, 1), wb(1, 1, 3))),
            "a": lambda: _dot(xa(0, 2, 0), wb(2, 0, 0)),
            "b": lambda: _dot(xa(0, 2, 1), wb(2, 1, 0)),
            "c": lambda: _dot(xa(1, 2, 0), wb(2, 0, 1)),
            "d": lambda: _dot(xa(1, 2, 1), wb(2, 1, 1)),
        }
        uses = {"1": ((0, 1), (3, 1)), "2": ((2, 1), (3, -1)), "3": ((1, 1), (3, 1)), "4": ((0, 1), (2, 1)),
                "5": ((0, -1), (1, 1)), "6": ((3, 1),), "7": ((0, 1),),
                "a": ((0, 1),), "b": ((1, 1),), "c": ((2, 1),), "d": ((3, 1),)}
        need = [5, 3, 3, 5]
        pend = [[], [], [], []]
        for t in Q_ORDER:
            m = prods[t]()
            for st, sg in uses[t]:
                pend[st].append((m, sg))
                if len(pend[st]) == need[st]:
                    tot = combine(pend[st])
                    store_q(st, tot)

    def oproj_group(g0, ws, order, last=False, static_out=False):
        zz = [zs[0], zs[1], zs[2], zs[3], zs[4]]
        zw = [0, zs[0], zs[1], zs[2]]

        def emit(g, c0, c1, val):
            tot = acc_ref[g, :, c0:c1] + val
            if last:
                o_stage[g, :, c0:c1] = tot.astype(o_stage.dtype)
                if static_out:
                    o_part(g, c0, c1).start()
            else:
                acc_ref[g, :, c0:c1] = tot

        def oa(i, k, v):
            return o_ref[2 * i + k + (0 if static_out else zz[v])]

        def wb(k, j, v):
            return wo_buf[ws + zw[v], k * W:(k + 1) * W, j * kh:min((j + 1) * kh, d_model)]

        bf = lambda v: v.astype(BF16)
        prods = {
            "1": lambda: _dot(bf(oa(0, 0, 0) + oa(1, 1, 0)), _add(wb(0, 0, 0), wb(1, 1, 0))),
            "2": lambda: _dot(bf(oa(1, 0, 0) + oa(1, 1, 1)), wb(0, 0, 1)),
            "3": lambda: _dot(bf(oa(0, 0, 1)), _sub(wb(0, 1, 0), wb(1, 1, 1))),
            "4": lambda: _dot(bf(oa(1, 1, 2)), _sub(wb(1, 0, 0), wb(0, 0, 2))),
            "5": lambda: _dot(bf(oa(0, 0, 2) + oa(0, 1, 0)), wb(1, 1, 2)),
            "6": lambda: _dot(bf(oa(1, 0, 1) - oa(0, 0, 3)), _add(wb(0, 0, 3), wb(0, 1, 1))),
            "7": lambda: _dot(bf(oa(0, 1, 1) - oa(1, 1, 3)), _add(wb(1, 0, 1), wb(1, 1, 3))),
            "a": lambda: _dot(bf(jnp.concatenate([oa(0, 0, 4), oa(0, 1, 2)], axis=1)), wo_buf[ws, :, 2 * kh:]),
            "b": lambda: _dot(bf(jnp.concatenate([oa(1, 0, 2), oa(1, 1, 4)], axis=1)), wo_buf[ws + zw[1], :, 2 * kh:]),
        }
        uses = {"1": ((0, 1), (3, 1)), "2": ((2, 1), (3, -1)), "3": ((1, 1), (3, 1)), "4": ((0, 1), (2, 1)),
                "5": ((0, -1), (1, 1)), "6": ((3, 1),), "7": ((0, 1),), "a": ((4, 1),), "b": ((5, 1),)}
        need = [4, 2, 2, 4, 1, 1]
        dest = [(0, 0), (0, 1), (1, 0), (1, 1), (0, 2), (1, 2)]
        pend = [[] for _ in need]
        for t in order:
            m = prods[t]()
            for st, sg in uses[t]:
                pend[st].append((m, sg))
                if len(pend[st]) == need[st]:
                    tot = combine(pend[st])
                    bi, jj = dest[st]
                    emit(g0 + bi, jj * kh, min((jj + 1) * kh, d_model), tot)
        if last and not static_out:
            for g in (g0, g0 + 1):
                o_stage[g, :, 0:2 * kh] = acc_ref[g, :, 0:2 * kh].astype(o_stage.dtype)
            o_copy(g0).start()
            o_copy(g0 + 1).start()

    def attend(slot, st, z0, z1):
        bi, r = st >> 1, (st & 1) * W
        if not isinstance(st, int):
            r = pl.multiple_of(r, 128)

        def rows(a, n):
            return pl.ds(r + a, n)

        def qk(h, order):
            zz = [0, zs[2], zs[3]] if h == 0 else [zs[5], zs[6], zs[7]]
            cw = 128
            half = kv_buf.shape[4] // 2

            def kb(d, j, c, v):
                return kv_buf[slot + zz[v], 0, bi, rows((h + d) * 128, 128), j * half + c:j * half + c + cw]

            def qa(m):
                if m % 2:
                    return q_ref[st, 0:128, h * 512 + (m // 2) * 128:h * 512 + (m // 2 + 1) * 128]
                return q_ref[st, 128:, h * 512 + (m // 2 - 1) * 128:h * 512 + (m // 2) * 128]

            def prod(t, c):
                return {
                    1: lambda: _dot(qa(1), _add(kb(0, 0, c, 0), kb(1, 1, c, 0))),
                    2: lambda: _dot(qa(2), kb(0, 0, c, 1)),
                    3: lambda: _dot(qa(3), _sub(kb(0, 1, c, 0), kb(1, 1, c, 1))),
                    4: lambda: _dot(qa(4), _sub(kb(1, 0, c, 0), kb(0, 0, c, 0))),
                    5: lambda: _dot(qa(5), kb(1, 1, c, 2)),
                    6: lambda: _dot(qa(6), _add(kb(0, 0, c, 0), kb(0, 1, c, 1))),
                    7: lambda: _dot(qa(7), _add(kb(1, 0, c, 1), kb(1, 1, c, 2))),
                }[t]()

            cs = list(range(0, half, cw))
            m = {}
            for phase in order:
                for c in cs:
                    for t in phase:
                        m[int(t), c] = prod(int(t), c)
            c11, c12, c21, c22 = [], [], [], []
            for c in cs:
                w_ = jnp.concatenate([m[1, c][0:r2] + m[4, c], m[1, c][r2:]], axis=0)
                c11.append(w_ + (m[7, c] - m[5, c]))
                c22.append(m[1, c][0:r2] - m[2, c] + m[6, c] + m[3, c][0:r2])
                c12.append(m[3, c] + m[5, c])
                c21.append(m[2, c] + m[4, c])
            return jnp.concatenate([jnp.concatenate(c11 + c12, axis=1), jnp.concatenate(c21 + c22, axis=1)], axis=0)

        def pv(h, s):
            pb, l = _softmax(s)
            pr = (pa_ref, pb_ref)[h]
            pr[z0] = pb
            sk = kv_buf.shape[4]

            def own(k0, k1):
                return lax.dot_general(pr[z1, :, k0:k1], kv_buf[slot, 1, bi, rows(h * 256, 128), k0:k1], NT,
                                       preferred_element_type=F32)

            def shared(k0, k1):
                return lax.dot_general(kv_buf[slot, 1, bi, rows(128 + h * 64, 64), k0:k1],
                                       pr[zs[2], :, k0:k1], NT, preferred_element_type=F32)

            ot = shared(0, sk // 2)
            od = own(0, sk // 2)
            ot = ot + shared(sk // 2, sk)
            od = od + own(sk // 2, sk)
            return od, ot, _rcp(l)

        def fin(ra, rb):
            od_a, ot_a, ia = ra
            od_b, ot_b, ib = rb
            om = jnp.concatenate([ot_a, ot_b], axis=0).T
            o_ref[st] = jnp.concatenate([od_a * ia, om * jnp.where(lane < 64, ia, ib), od_b * ib], axis=1)

        return qk, pv, fin

    def attend_seq(slot, sts, z0, z1, filler=None):
        parts = [attend(slot, st, z0, z1) for st in sts]
        n = 2 * len(sts)
        s = {}
        r = {}
        seq = ["K0"]
        for u in range(n):
            if u + 1 < n:
                seq.append("K%d" % (u + 1))
            seq.append("P%d" % u)
        for tok in seq:
            u = int(tok[1:])
            qk, pv, fin = parts[u // 2]
            if tok == "K1" and filler is not None:
                filler()
            if tok[0] == "K":
                s[u] = qk(u % 2, K_ORDER if u else K_ORDER_FIRST)
            else:
                r[u] = pv(u % 2, s[u])
                if u % 2 == 1:
                    fin(r[u - 1], r[u])

    def kv(i):
        return [functools.partial(kv_step, 0, i, kv_sem.at[i]), functools.partial(kv_step, 1, i, kv_sem.at[i])]

    def xs(*gs):
        return [functools.partial(x_copy, g) for g in gs]

    def start(mks):
        for mk in mks:
            mk().start()

    def wait(mks):
        for mk in mks:
            mk().wait()

    def fence():
        pl.semaphore_signal(f_sem, 1)
        pl.semaphore_wait(f_sem, 1)

    wq00, wq01 = [functools.partial(wq_copy, 0, 0)], [functools.partial(wq_copy, 0, 1)]
    wo0 = [functools.partial(wo_copy, 0)]
    w1 = [functools.partial(wq_copy, 1, 0), functools.partial(wq_copy, 1, 1), functools.partial(wo_copy, 1)]
    for i in range(8):
        zs[i] = 0

    def at(i, table, fn):
        for key, mks in table.items():
            if mks:
                pl.when(i == key)(functools.partial(fn, mks))

    for group in (xs(0) + wq00, xs(1), wq01, kv(0) + kv(1) + kv(2) + kv(3), xs(2, 3), wo0,
                  kv(4) + kv(5) + kv(6) + kv(7), xs(4, 5)):
        start(group)
        fence()

    def zero_body(g, carry):
        acc_ref[g] = jnp.zeros(acc_ref.shape[1:], F32)
        return carry

    lax.fori_loop(0, nb, zero_body, 0)

    def q0_body(i, carry):
        at(i, {0: xs(0) + wq00, 1: xs(1), 2: wq01}, wait)
        g = jnp.bitwise_and(i, 1)
        pi = lax.shift_right_logical(i, 1)
        store_q(2 * g + pi, _dot(x_buf[g], wq_buf[0, pi]))
        return carry

    lax.fori_loop(0, 4, q0_body, 0)

    def ramp_body(i, carry):
        slot = lax.shift_right_logical(i, 2)
        st = jnp.bitwise_and(i, 3)
        for which in range(2):
            dst = kv_buf.at[slot, which, lax.shift_right_logical(st, 1),
                            pl.ds(pl.multiple_of(jnp.bitwise_and(st, 1) * W, 128), W)]
            pltpu.make_async_copy(dst, dst, kv_sem.at[i]).wait()
        attend_seq(slot, [st], zs[0], zs[1])

        @pl.when(st == 3)
        def _():
            kv_body(0, slot + 2).start()
            kv_body(1, slot + 2).start()
            at(i, {3: xs(2, 3) + wo0, 7: xs(4, 5)}, wait)
            at(i, {3: xs(6, 7), 7: w1}, start)
            fence()
            qproj_group(2 * slot + 2, 0)
            oproj_group(2 * slot, 0, O_ORDER)
            pl.when(i == 3)(lambda: oproj_group(0, 0, O_ORDER_TAIL))
        return carry

    lax.fori_loop(0, 8, ramp_body, 0)
    wait(xs(6, 7))

    def fast_body(mode, it, carry):
        gg = lax.shift_right_logical(it, lg_ni)
        j = jnp.bitwise_and(it, ni - 1)
        slot = jnp.bitwise_and(it, 1)
        last_j = j == ni - 1
        pltpu.make_async_copy(kv_buf.at[slot], kv_buf.at[slot], body_sem.at[slot]).wait()
        if mode == "mid":
            @pl.when(last_j)
            def _():
                wq_copy(gg + 1, 0).wait()
                wq_copy(gg + 1, 1).wait()
                wo_copy(gg + 1).wait()

        z0, z1 = zs[0], zs[1]
        pit = it - 1
        attend_seq(slot, [0, 1, 2, 3], z0, z1,
                   lambda: oproj_group(2 * jnp.bitwise_and(pit, ni - 1),
                                       jnp.bitwise_and(lax.shift_right_logical(pit, lg_ni), 1), O_ORDER_TAIL,
                                       mode != "mid"))
        if mode != "final":
            gq = jnp.minimum(lax.shift_right_logical(it + 1, lg_ni), ngroup - 1)
            qproj_group(2 * jnp.bitwise_and(it + 1, ni - 1), jnp.bitwise_and(gq, 1))
        if mode == "final":
            oproj_group(nb - 2, (ngroup - 1) & 1, O_ORDER_FINAL, True, True)
        else:
            oproj_group(2 * j, jnp.bitwise_and(gg, 1), O_ORDER)

        if mode != "final":
            @pl.when(it + 2 < nbody)
            def _():
                kv_body(0, it + 2).start()
                kv_body(1, it + 2).start()

        if mode == "mid":
            @pl.when(jnp.logical_and(last_j, gg + 2 < ngroup))
            def _():
                wq_copy(gg + 2, 0).start()
                wq_copy(gg + 2, 1).start()

            @pl.when(jnp.logical_and(j == 0, gg + 1 < ngroup))
            def _():
                wo_copy(gg + 1).start()
        return carry

    lax.fori_loop(2, nbody - ni + 1, functools.partial(fast_body, "mid"), 0)
    lax.fori_loop(nbody - ni + 1, nbody - 1, functools.partial(fast_body, "last"), 0)
    fast_body("final", jnp.int32(nbody - 1), 0)
    for g in range(nb):
        o_copy(g).wait()


@jax.jit
def pallas_standalone__gqa_block_cached__near_ridge_kernel(x, k_cache, v_cache, wq, wo):
    B, Sq, D = x.shape
    _, Hkv, Sk, Dh = k_cache.shape
    kt = jnp.swapaxes(k_cache, 2, 3).reshape(B, Hkv * Dh, Sk)
    vt = jnp.swapaxes(v_cache, 2, 3).reshape(B, Hkv * Dh, Sk)
    scale = (Dh ** -0.5) * math.log2(math.e)
    ngroup = Hkv // 4
    any_spec = pl.BlockSpec(memory_space=pl.ANY)
    return pl.pallas_call(
        functools.partial(_kernel, scale=scale, sq=Sq, nb=B, ngroup=ngroup),
        grid=(1,),
        in_specs=[any_spec] * 5,
        out_specs=any_spec,
        out_shape=jax.ShapeDtypeStruct((B, Sq, D), x.dtype),
        scratch_shapes=[
            pltpu.VMEM((B, Sq, D), BF16),
            pltpu.VMEM((2, 2, 2, GW, Sk), BF16),
            pltpu.VMEM((2, 2, D, W), BF16),
            pltpu.VMEM((2, GW, D), BF16),
            pltpu.VMEM((B, Sq, D), F32),
            pltpu.VMEM((4, Sq, 1024), BF16),
            pltpu.VMEM((B, Sq, D), BF16),
            pltpu.VMEM((1, Sq, Sk), BF16),
            pltpu.VMEM((1, Sq, Sk), BF16),
            pltpu.VMEM((4, Sq, W), F32),
            pltpu.SMEM((8,), jnp.int32),
            pltpu.SemaphoreType.DMA((B,)),
            pltpu.SemaphoreType.DMA((8,)),
            pltpu.SemaphoreType.DMA((2,)),
            pltpu.SemaphoreType.REGULAR,
            pltpu.SemaphoreType.DMA((3, 2)),
            pltpu.SemaphoreType.DMA((B,)),
        ],
        compiler_params=pltpu.CompilerParams(
            dimension_semantics=("arbitrary",),
            vmem_limit_bytes=100 * 1024 * 1024,
            disable_bounds_checks=True,
        ),
    )(x, kt, vt, wq, wo)
```
